```python
import jax
import jax.numpy as jnp

def _softmax(x, axis=-1):
    return jax.nn.softmax(x, axis=axis)

def _gelu(x):
    return jax.nn.gelu(x, approximate=True)

def _silu(x):
    return jax.nn.silu(x)

def _sigmoid(x):
    return jax.nn.sigmoid(x)

def _layernorm(x, axis=-1, eps=1e-05):
    m = jnp.mean(x, axis=axis, keepdims=True)
    v = jnp.var(x, axis=axis, keepdims=True)
    return (x - m) / jnp.sqrt(v + eps)

def _scatter_add(tgt, idx, src, axis=0):
    return tgt.at[idx].add(src)

def _segment_sum(src, seg, n):
    return jax.ops.segment_sum(src, seg, n)

class _Rng:

    def __init__(self, key):
        self._k = key

    def _next(self):
        self._k, sub = jax.random.split(self._k)
        return sub

    def normal(self, shape):
        return jax.random.normal(self._next(), shape, dtype=jnp.bfloat16)

    def randint(self, lo, hi, shape):
        return jax.random.randint(self._next(), shape, lo, hi, dtype=jnp.int32)

    def uniform(self, shape, lo=0.0, hi=1.0):
        return jax.random.uniform(self._next(), shape, jnp.bfloat16, lo, hi)

    def permutation(self, n):
        return jax.random.permutation(self._next(), n)
kernel_name = 'adaLN_cond__ssm_conv_h3__mixer_s_mlp__prompt'

def setup_inputs():
    _rng = _Rng(jax.random.key(int.from_bytes(__import__("os").urandom(4), "little")))
    _w = lambda a: (lambda t: t.astype(jnp.bfloat16) if jnp.issubdtype(t.dtype, jnp.floating) else t)(jnp.asarray(a))

    def _A_setup():
        B, S, D = (1, 2048, 640)
        ks = 4
        return {'q': _w((lambda *s: _rng.normal(s) * 0.05)(B, S, D)), 'k': _w((lambda *s: _rng.normal(s) * 0.05)(B, S, D)), 'v': _w((lambda *s: _rng.normal(s) * 0.05)(B, S, D)), 'shift_k': _w((lambda *s: _rng.normal(s) * 0.05)(D, ks) * 0.5), 'ssm_k': _w((lambda *s: _rng.normal(s) * 0.05)(D, S) * (1.0 / S ** 0.5)), 'ssm_D': _w((lambda *s: _rng.normal(s) * 0.05)(D))}
    _A_in = _A_setup()

    def _B_setup():
        B, S, D, F = (1, 2048, 640, 1728)
        return {'x': _w((lambda *s: _rng.normal(s) * 0.05)(B, S, D)), 'w1': _w((lambda *s: _rng.normal(s) * 0.05)(D, D) * D ** (-0.5)), 'w2': _w((lambda *s: _rng.normal(s) * 0.05)(D, D) * D ** (-0.5)), 'w3': _w((lambda *s: _rng.normal(s) * 0.05)(D, F) * D ** (-0.5)), 'w4': _w((lambda *s: _rng.normal(s) * 0.05)(F, D) * F ** (-0.5))}
    _B_in = _B_setup()
    return {'A_q': _A_in['q'], 'A_k': _A_in['k'], 'A_v': _A_in['v'], 'A_shift_k': _A_in['shift_k'], 'A_ssm_k': _A_in['ssm_k'], 'A_ssm_D': _A_in['ssm_D'], 'B_x': _B_in['x'], 'B_w1': _B_in['w1'], 'B_w2': _B_in['w2'], 'B_w3': _B_in['w3'], 'B_w4': _B_in['w4'], 'c': _w((lambda *s: _rng.normal(s) * 0.05)(1, 640)), 'w_mod': _w((lambda *s: _rng.normal(s) * 0.05)(640, 6 * 640) * 640 ** (-0.5))}

def reference(A_q, A_k, A_v, A_shift_k, A_ssm_k, A_ssm_D, B_x, B_w1, B_w2, B_w3, B_w4, c, w_mod):

    def _A_ref(q, k, v, shift_k, ssm_k, ssm_D):
        B, S, D = q.shape
        ks = shift_k.shape[-1]
        k_pad = jnp.pad(k, ((0, 0), (ks - 1, 0), (0, 0)))
        k_shift = jnp.zeros_like(k)
        for t in range(ks):
            k_shift = k_shift + k_pad[:, t:t + S, :] * shift_k[:, ks - 1 - t][None, None, :]
        kv = k_shift * v
        L = 2 * S
        kv_pad = jnp.pad(kv, ((0, 0), (0, S), (0, 0)))
        kf_pad = jnp.pad(ssm_k, ((0, 0), (0, S)))
        kv_f = (lambda x, axes=(-2, -1): jnp.fft.rfft2(x.astype(jnp.float32), axes=axes))(kv_pad[:, None, :, :], axes=(1, 2))
        kf_f = (lambda x, axes=(-2, -1): jnp.fft.rfft2(x.astype(jnp.float32), axes=axes))(kf_pad[:, None, :], axes=(1, 2))
        kf_f = (lambda x, *d: x.transpose(*d))(kf_f, 1, 2, 0)
        y_f = kv_f * kf_f[None, :, :, :]
        y = (lambda x, s, axes=(-2, -1): jnp.fft.irfft2(x, s=s, axes=axes).astype(jnp.bfloat16))(y_f, (1, L), axes=(1, 2))[:, 0, :S, :]
        y = y + kv * ssm_D[None, None, :]
        return q * y

    def _B_ref(x, w1, w2, w3, w4):
        B, S, D = x.shape
        h = _gelu(_layernorm(x, axis=-1) @ w1)
        c = D // 4
        g0 = jnp.pad(h[:, :, 0 * c:1 * c], ((0, 0), (1, 0), (0, 0)))[:, :S, :]
        g1 = jnp.pad(h[:, :, 1 * c:2 * c], ((0, 0), (0, 1), (0, 0)))[:, 1:, :]
        g2 = jnp.pad(h[:, :, 2 * c:3 * c], ((0, 0), (2, 0), (0, 0)))[:, :S, :]
        g3 = jnp.pad(h[:, :, 3 * c:], ((0, 0), (0, 2), (0, 0)))[:, 2:, :]
        hs = jnp.concatenate([g0, g1, g2, g3], axis=-1) @ w2
        x1 = x + hs
        h2 = _gelu(_layernorm(x1, axis=-1) @ w3) @ w4
        return x1 + h2
    x = A_q
    mod = (_silu(c) @ w_mod).reshape(c.shape[0], 6, 1, -1)
    sa, ca, ga, sb, cb, gb = (mod[:, 0].copy(), mod[:, 1].copy(), mod[:, 2].copy(), mod[:, 3].copy(), mod[:, 4].copy(), mod[:, 5].copy())
    h = _layernorm(x, axis=-1) * (1 + ca) + sa
    x = x + ga * _A_ref(h, A_k, A_v, A_shift_k, A_ssm_k, A_ssm_D)
    h = _layernorm(x, axis=-1) * (1 + cb) + sb
    x = x + gb * _B_ref(h, B_w1, B_w2, B_w3, B_w4)
    return x
```

```python
import numpy as np
import jax
import jax.numpy as jnp
import jax.experimental.pallas as pl
import jax.experimental.pallas.tpu as pltpu

S, D, F = 2048, 640, 1728
C = 128
NC = S // C
NG = D // 128
TM = 256
NT = S // TM
PAD = 8
F32, BF16 = jnp.float32, jnp.bfloat16


def _dft_consts():
    w = 2.0 * np.pi * (np.arange(C) + 0.5) / (2 * C)
    t = np.arange(2 * C)
    a = w[:, None] * t[None, :]
    fk = np.concatenate([np.cos(a), -np.sin(a)], axis=0)
    an = t[C:, None] * w[None, :]
    inv = np.concatenate([np.cos(an), -np.sin(an)], axis=1) / C
    sgn = -np.sin(w * C)[:, None] * np.ones((1, 128))
    return fk, inv, sgn


def _ln(x):
    m = jnp.mean(x, axis=-1, keepdims=True)
    xc = x - m
    v = jnp.mean(xc * xc, axis=-1, keepdims=True)
    return xc * jax.lax.rsqrt(v + 1e-5)


def _gelu(x):
    return jax.nn.gelu(x, approximate=True)


def _dot(a, b):
    return jnp.dot(a, b, preferred_element_type=F32)


def _kernel(q_h, k_h, v_h, sk_ref, ssmk_h, sd_ref, w1_h, w2_h, w3_h, w4_h, c_ref, wm_h,
            fk_ref, inv_ref, sgn_ref, o_h,
            q_v, k_v, v_v, ssmk_v, w1_v, w2_v, w3_v, w4_v, wm_v, o_v,
            kf_s, xf_s, kfreq_s, yf_s, y_s, h_s, sems, osems):
    srcs = [ssmk_h, k_h, v_h, wm_h, q_h, w1_h, w2_h, w3_h, w4_h]
    dsts = [ssmk_v, k_v, v_v, wm_v, q_v, w1_v, w2_v, w3_v, w4_v]
    cps = [pltpu.make_async_copy(s, d, sems.at[i]) for i, (s, d) in enumerate(zip(srcs, dsts))]
    for cp in cps:
        cp.start()
    c_ssmk, c_k, c_v, c_wm, c_q, c_w1, c_w2, c_w3, c_w4 = cps

    sk = jnp.transpose(sk_ref[...].astype(F32))
    sd = sd_ref[...].astype(F32)
    fk = fk_ref[...]
    fx = fk_ref[:, 0:C]
    fb = fk_ref[:, C:2 * C]
    inv = inv_ref[...]
    nt = (((1,), (1,)), ((), ()))

    c_ssmk.wait()
    c_k.wait()
    c_v.wait()

    for g in range(NG):
        ls = slice(g * 128, (g + 1) * 128)
        kf_s[0:PAD, :] = jnp.zeros((PAD, 128), F32)
        kf_s[PAD:, :] = k_v[:, ls].astype(F32)
        for j in range(NC):
            r0 = j * C
            ks = kf_s[PAD + r0:PAD + r0 + C, :] * sk[0:1, ls]
            for s in range(1, 4):
                ks = ks + kf_s[PAD + r0 - s:PAD + r0 - s + C, :] * sk[s:s + 1, ls]
            kv = ks * v_v[r0:r0 + C, ls].astype(F32)
            xf_s[j] = _dot(fx, kv.astype(BF16))
            if j == 0:
                kfr = jax.lax.dot_general(fb, ssmk_v[ls, 0:C], nt, preferred_element_type=F32)
                kfreq_s[0, 0:C, :] = kfr[0:C]
                kfreq_s[0, C:, :] = kfr[C:] + sgn_ref[...] * sd[:, ls]
            else:
                kfreq_s[j] = jax.lax.dot_general(
                    fk, ssmk_v[ls, (j - 1) * C:(j + 1) * C], nt, preferred_element_type=F32)

        def conv(p, carry):
            re = pl.ds(pl.multiple_of(p * 16, 16), 16)
            im = pl.ds(pl.multiple_of(C + p * 16, 16), 16)
            for i in range(NC):
                ar = ai = None
                for j in range(i + 1):
                    xr, xi = xf_s[j, re, :], xf_s[j, im, :]
                    kr, ki = kfreq_s[i - j, re, :], kfreq_s[i - j, im, :]
                    tr = xr * kr - xi * ki
                    ti = xr * ki + xi * kr
                    ar = tr if ar is None else ar + tr
                    ai = ti if ai is None else ai + ti
                yf_s[i, re, :] = ar.astype(BF16)
                yf_s[i, im, :] = ai.astype(BF16)
            return carry

        jax.lax.fori_loop(0, C // 16, conv, 0)
        for i in range(NC):
            y_s[i * C:(i + 1) * C, ls] = _dot(inv, yf_s[i]).astype(BF16)

    c_wm.wait()
    cs = jax.nn.silu(c_ref[...].astype(F32)).astype(BF16)
    mod = _dot(jnp.broadcast_to(cs, (16, D)), wm_v[...])[0:1]
    sa, ca, ga, sb, cb, gb = [mod[:, i * D:(i + 1) * D] for i in range(6)]

    for cp in (c_q, c_w1, c_w2, c_w3, c_w4):
        cp.wait()

    for g in range(NG):
        h_s[g, 0:PAD, :] = jnp.zeros((PAD, 128), F32)
        h_s[g, PAD + S:, :] = jnp.zeros((PAD, 128), F32)

    def x1_hb(rows):
        q = q_v[rows, :].astype(F32)
        h = _ln(q) * (1.0 + ca) + sa
        x1 = q + ga * (h * y_s[rows, :].astype(F32))
        return x1, _ln(x1) * (1.0 + cb) + sb

    def b1(t, carry):
        r0 = pl.multiple_of(t * TM, TM)
        _, hb = x1_hb(pl.ds(r0, TM))
        h = _gelu(_dot(_ln(hb).astype(BF16), w1_v[...]))
        for g in range(NG):
            h_s[g, pl.ds(PAD + r0, TM), :] = h[:, g * 128:(g + 1) * 128]
        return carry

    jax.lax.fori_loop(0, NT, b1, 0)

    def out_cp(t):
        r0 = pl.multiple_of(t * TM, TM)
        return pltpu.make_async_copy(o_v.at[pl.ds(r0, TM)], o_h.at[pl.ds(r0, TM)], osems.at[t])

    lane = jax.lax.broadcasted_iota(jnp.int32, (TM, 128), 1)

    def b2(t, carry):
        r0 = pl.multiple_of(t * TM, TM)
        x1, hb = x1_hb(pl.ds(r0, TM))
        ld = lambda g, off: h_s[g, pl.ds(PAD + r0 + off, TM), :]
        hs = jnp.concatenate([
            ld(0, -1),
            jnp.where(lane < 32, ld(1, -1), ld(1, 1)),
            jnp.where(lane < 64, ld(2, 1), ld(2, -2)),
            jnp.where(lane < 96, ld(3, -2), ld(3, 2)),
            ld(4, 2)], axis=1)
        xb = hb + _dot(hs.astype(BF16), w2_v[...])
        u = _gelu(_dot(_ln(xb).astype(BF16), w3_v[...]))
        h2 = _dot(u.astype(BF16), w4_v[...])
        o_v[pl.ds(r0, TM), :] = (x1 + gb * (xb + h2)).astype(BF16)
        out_cp(t).start()
        return carry

    jax.lax.fori_loop(0, NT, b2, 0)
    for t in range(NT):
        out_cp(t).wait()


@jax.jit
def pallas_adaLN_cond__ssm_conv_h3__mixer_s_mlp__prompt_kernel(
    A_q, A_k, A_v, A_shift_k, A_ssm_k, A_ssm_D, B_x, B_w1, B_w2, B_w3, B_w4, c, w_mod,
):
    fk, inv, sgn = _dft_consts()
    hbm = pl.BlockSpec(memory_space=pl.ANY)
    vm = pl.BlockSpec(memory_space=pltpu.VMEM)
    V = pltpu.VMEM
    out = pl.pallas_call(
        _kernel,
        in_specs=[hbm, hbm, hbm, vm, hbm, vm, hbm, hbm, hbm, hbm, vm, hbm, vm, vm, vm],
        out_specs=hbm,
        out_shape=jax.ShapeDtypeStruct((S, D), BF16),
        scratch_shapes=[
            V((S, D), BF16), V((S, D), BF16), V((S, D), BF16), V((D, S), BF16),
            V((D, D), BF16), V((D, D), BF16), V((D, F), BF16), V((F, D), BF16),
            V((D, 6 * D), BF16), V((S, D), BF16),
            V((PAD + S, 128), F32), V((NC, 2 * C, 128), F32), V((NC, 2 * C, 128), F32),
            V((NC, 2 * C, 128), BF16), V((S, D), BF16), V((NG, S + 2 * PAD, 128), F32),
            pltpu.SemaphoreType.DMA((9,)), pltpu.SemaphoreType.DMA((NT,)),
        ],
        compiler_params=pltpu.CompilerParams(vmem_limit_bytes=100 * 1024 * 1024),
    )(A_q.reshape(S, D), A_k.reshape(S, D), A_v.reshape(S, D), A_shift_k, A_ssm_k,
      A_ssm_D.reshape(1, D), B_w1, B_w2, B_w3, B_w4, c, w_mod,
      jnp.asarray(fk, BF16), jnp.asarray(inv, BF16), jnp.asarray(sgn, F32))
    return out.reshape(1, S, D)
```

```python
import numpy as np
import jax
import jax.numpy as jnp
import jax.experimental.pallas as pl
import jax.experimental.pallas.tpu as pltpu

S, D, F = 2048, 640, 1728
C = 128
NC = S // C
NG = D // 128
TM = 256
NT = S // TM
PAD = 8
F32, BF16 = jnp.float32, jnp.bfloat16


def _dft_consts():
    w = 2.0 * np.pi * (np.arange(C) + 0.5) / (2 * C)
    t = np.arange(2 * C)
    a = w[:, None] * t[None, :]
    fk = np.concatenate([np.cos(a), -np.sin(a)], axis=0)
    an = t[C:, None] * w[None, :]
    inv = np.concatenate([np.cos(an), -np.sin(an)], axis=1) / C
    sgn = -np.sin(w * C)[:, None] * np.ones((1, 128))
    return fk, inv, sgn


def _ln(x):
    m = jnp.mean(x, axis=-1, keepdims=True)
    xc = x - m
    v = jnp.mean(xc * xc, axis=-1, keepdims=True)
    return xc * jax.lax.rsqrt(v + 1e-5)


def _gelu(x):
    return jax.nn.gelu(x, approximate=True)


def _dot(a, b):
    return jnp.dot(a, b, preferred_element_type=F32)


def _kernel(q_h, k_h, v_h, sk_ref, ssmk_h, sd_ref, w1_h, w2_h, w3_h, w4_h, c_ref, wm_h,
            fk_ref, inv_ref, sgn_ref, o_h,
            q_v, k_v, v_v, ssmk_v, w1_v, w2_v, w3_v, w4_v, wm_v, o_v,
            kf_s, xf0, xf1, kq0, kq1, yf0, yf1, y_s, h_s, sems, osems):
    xf_s, kfreq_s, yf_s = (xf0, xf1), (kq0, kq1), (yf0, yf1)
    ssmk_v[:, 0:C] = jnp.zeros((D, C), BF16)
    lsl = lambda g: slice(g * 128, (g + 1) * 128)
    a_cps = [[pltpu.make_async_copy(k_h.at[:, lsl(g)], k_v.at[:, lsl(g)], sems.at[3 * g]),
              pltpu.make_async_copy(v_h.at[:, lsl(g)], v_v.at[:, lsl(g)], sems.at[3 * g + 1]),
              pltpu.make_async_copy(ssmk_h.at[lsl(g), :], ssmk_v.at[lsl(g), C:], sems.at[3 * g + 2])]
             for g in range(NG)]
    srcs = [wm_h, q_h, w1_h, w2_h, w3_h, w4_h]
    dsts = [wm_v, q_v, w1_v, w2_v, w3_v, w4_v]
    cps = [pltpu.make_async_copy(s, d, sems.at[3 * NG + i]) for i, (s, d) in enumerate(zip(srcs, dsts))]
    c_wm, c_q, c_w1, c_w2, c_w3, c_w4 = cps
    for cp in a_cps[0] + a_cps[1]:
        cp.start()

    sk = sk_ref[...].astype(F32)
    sd = sd_ref[...].astype(F32)
    fk = fk_ref[...]
    fx = fk_ref[:, 0:C]
    fb = fk_ref[:, C:2 * C]
    inv = inv_ref[...]
    nt = (((1,), (1,)), ((), ()))

    kf_s[0:PAD, :] = jnp.zeros((PAD, 128), F32)

    def fwd(g, j):
        ls, b = lsl(g), g % 2
        r0 = j * C if isinstance(j, int) else pl.multiple_of(j * C, C)
        kf_s[pl.ds(PAD + r0, C), :] = k_v[pl.ds(r0, C), ls].astype(F32)
        ks = kf_s[pl.ds(PAD + r0, C), :] * sk[0:1, ls]
        for s in range(1, 4):
            ks = ks + kf_s[pl.ds(PAD + r0 - s, C), :] * sk[s:s + 1, ls]
        kv = ks * v_v[pl.ds(r0, C), ls].astype(F32)
        xf_s[b][j] = _dot(fx, kv.astype(BF16))
        kfreq_s[b][j] = jax.lax.dot_general(
            fk, ssmk_v[ls, pl.ds(r0, 2 * C)], nt, preferred_element_type=F32)

    def add_d(g):
        kfreq_s[g % 2][0, C:, :] = kfreq_s[g % 2][0, C:, :] + sgn_ref[...] * sd[:, lsl(g)]

    def invf(g, i):
        r0 = i * C if isinstance(i, int) else pl.multiple_of(i * C, C)
        y_s[pl.ds(r0, C), lsl(g)] = _dot(inv, yf_s[g % 2][i]).astype(BF16)

    for cp in a_cps[0]:
        cp.wait()
    for j in range(NC):
        fwd(0, j)

    for g in range(NG):
        add_d(g)
        if g + 2 < NG:
            for cp in a_cps[g + 2]:
                cp.start()
        if g == 1:
            c_wm.start()
            c_q.start()
        if g == 3:
            for cp in (c_w1, c_w2, c_w3, c_w4):
                cp.start()
        if g + 1 < NG:
            for cp in a_cps[g + 1]:
                cp.wait()

        def conv(p, carry, g=g):
            b = g % 2
            re = pl.ds(pl.multiple_of(p * 16, 16), 16)
            im = pl.ds(pl.multiple_of(C + p * 16, 16), 16)
            G = 2
            for i0 in range(0, NC, G):
                if g + 1 < NG and i0 == 6:
                    fwd(g + 1, 2 * p)
                if g + 1 < NG and i0 == 10:
                    fwd(g + 1, 2 * p + 1)
                if g > 0 and i0 == 0:
                    invf(g - 1, 2 * p)
                if g > 0 and i0 == 2:
                    invf(g - 1, 2 * p + 1)
                acc = {}
                for j in range(i0 + G):
                    xr, xi = xf_s[b][j, re, :], xf_s[b][j, im, :]
                    for i in range(max(i0, j), i0 + G):
                        kr, ki = kfreq_s[b][i - j, re, :], kfreq_s[b][i - j, im, :]
                        if i in acc:
                            acc[i] = ((acc[i][0] + xr * kr) - xi * ki, (acc[i][1] + xr * ki) + xi * kr)
                        else:
                            acc[i] = (xr * kr - xi * ki, xr * ki + xi * kr)
                for i in acc:
                    yf_s[b][i, re, :] = acc[i][0].astype(BF16)
                    yf_s[b][i, im, :] = acc[i][1].astype(BF16)
            return carry

        with jax.named_scope('conv'):
            jax.lax.fori_loop(0, C // 16, conv, 0)
    for i in range(NC):
        invf(NG - 1, i)

    c_wm.wait()
    cs = jax.nn.silu(c_ref[...].astype(F32)).astype(BF16)
    mod = _dot(jnp.broadcast_to(cs, (16, D)), wm_v[...])[0:1]
    sa, ca, ga, sb, cb, gb = [mod[:, i * D:(i + 1) * D] for i in range(6)]

    for cp in (c_q, c_w1, c_w2, c_w3, c_w4):
        cp.wait()

    for g in range(NG):
        h_s[g, 0:PAD, :] = jnp.zeros((PAD, 128), F32)
        h_s[g, PAD + S:, :] = jnp.zeros((PAD, 128), F32)

    def x1_hb(rows):
        q = q_v[rows, :].astype(F32)
        h = _ln(q) * (1.0 + ca) + sa
        x1 = q + ga * (h * y_s[rows, :].astype(F32))
        return x1, _ln(x1) * (1.0 + cb) + sb

    def b1(t, carry):
        r0 = t * TM if isinstance(t, int) else pl.multiple_of(t * TM, TM)
        _, hb = x1_hb(pl.ds(r0, TM))
        h = _gelu(_dot(_ln(hb).astype(BF16), w1_v[...]))
        for g in range(NG):
            h_s[g, pl.ds(PAD + r0, TM), :] = h[:, g * 128:(g + 1) * 128]
        return carry

    with jax.named_scope('b1'):
        b1(0, 0)
        b1(1, 0)

    def out_cp(t):
        r0 = pl.multiple_of(t * TM, TM)
        return pltpu.make_async_copy(o_v.at[pl.ds(r0, TM)], o_h.at[pl.ds(r0, TM)], osems.at[t])

    lane = jax.lax.broadcasted_iota(jnp.int32, (TM, 128), 1)

    def b2(t, carry, ahead=True):
        r0 = pl.multiple_of(t * TM, TM)
        x1, hb = x1_hb(pl.ds(r0, TM))
        ld = lambda g, off: h_s[g, pl.ds(PAD + r0 + off, TM), :]
        hs = jnp.concatenate([
            ld(0, -1),
            jnp.where(lane < 32, ld(1, -1), ld(1, 1)),
            jnp.where(lane < 64, ld(2, 1), ld(2, -2)),
            jnp.where(lane < 96, ld(3, -2), ld(3, 2)),
            ld(4, 2)], axis=1)
        if ahead:
            b1(t + 2, 0)
        xb = hb + _dot(hs.astype(BF16), w2_v[...])
        u = _gelu(jax.lax.dot_general(_ln(xb).astype(BF16), w3_v[...], nt, preferred_element_type=F32))
        h2 = _dot(u.astype(BF16), w4_v[...])
        o_v[pl.ds(r0, TM), :] = (x1 + gb * (xb + h2)).astype(BF16)
        out_cp(t).start()
        return carry

    with jax.named_scope('b2'):
        jax.lax.fori_loop(0, NT - 2, b2, 0)
        jax.lax.fori_loop(NT - 2, NT, lambda t, c_: b2(t, c_, False), 0)
    for t in range(NT):
        out_cp(t).wait()


@jax.jit
def pallas_adaLN_cond__ssm_conv_h3__mixer_s_mlp__prompt_kernel(
    A_q, A_k, A_v, A_shift_k, A_ssm_k, A_ssm_D, B_x, B_w1, B_w2, B_w3, B_w4, c, w_mod,
):
    fk, inv, sgn = _dft_consts()
    hbm = pl.BlockSpec(memory_space=pl.ANY)
    vm = pl.BlockSpec(memory_space=pltpu.VMEM)
    V = pltpu.VMEM
    out = pl.pallas_call(
        _kernel,
        in_specs=[hbm, hbm, hbm, vm, hbm, vm, hbm, hbm, hbm, hbm, vm, hbm, vm, vm, vm],
        out_specs=hbm,
        out_shape=jax.ShapeDtypeStruct((S, D), BF16),
        scratch_shapes=[
            V((S, D), BF16), V((S, D), BF16), V((S, D), BF16), V((D, C + S), BF16),
            V((D, D), BF16), V((D, D), BF16), V((F, D), BF16), V((F, D), BF16),
            V((D, 6 * D), BF16), V((S, D), BF16),
            V((PAD + S, 128), F32), *[V((NC, 2 * C, 128), F32)] * 4,
            *[V((NC, 2 * C, 128), BF16)] * 2, V((S, D), BF16), V((NG, S + 2 * PAD, 128), F32),
            pltpu.SemaphoreType.DMA((3 * NG + 6,)), pltpu.SemaphoreType.DMA((NT,)),
        ],
        compiler_params=pltpu.CompilerParams(vmem_limit_bytes=100 * 1024 * 1024),
    )(A_q.reshape(S, D), A_k.reshape(S, D), A_v.reshape(S, D), A_shift_k.T, A_ssm_k,
      A_ssm_D.reshape(1, D), B_w1, B_w2, B_w3.T, B_w4, c, w_mod,
      jnp.asarray(fk, BF16), jnp.asarray(inv, BF16), jnp.asarray(sgn, F32))
    return out.reshape(1, S, D)
```

```python
import numpy as np
import jax
import jax.numpy as jnp
import jax.experimental.pallas as pl
import jax.experimental.pallas.tpu as pltpu

S, D, F = 2048, 640, 1728
C = 128
NC = S // C
NG = D // 128
TM = 256
NT = S // TM
PAD = 8
F32, BF16 = jnp.float32, jnp.bfloat16


def _dft_consts():
    w = 2.0 * np.pi * (np.arange(C) + 0.5) / (2 * C)
    t = np.arange(2 * C)
    a = w[:, None] * t[None, :]
    fk = np.concatenate([np.cos(a), -np.sin(a)], axis=0)
    an = t[C:, None] * w[None, :]
    inv = np.concatenate([np.cos(an), -np.sin(an)], axis=1) / C
    sgn = -np.sin(w * C)[:, None] * np.ones((1, 128))
    return fk, inv, sgn


def _ln(x):
    m = jnp.mean(x, axis=-1, keepdims=True)
    xc = x - m
    v = jnp.mean(xc * xc, axis=-1, keepdims=True)
    return xc * jax.lax.rsqrt(v + 1e-5)


def _gelu(x):
    return jax.nn.gelu(x, approximate=True)


def _dot(a, b):
    return jnp.dot(a, b, preferred_element_type=F32)


def _kernel(q_h, k_h, v_h, sk_ref, ssmk_h, sd_ref, w1_h, w2_h, w3_h, w4_h, c_ref, wm_h,
            fk_ref, inv_ref, sgn_ref, o_h,
            q_v, k_v, v_v, ssmk_v, w1_v, w2_v, w3_v, w4_v, wm_v, o_v,
            kf_s, xf_s, kq_s, yf_s, y_s, h_s, sems, osems):
    lsl = lambda g: slice(g * 128, (g + 1) * 128)
    a_cps = [[pltpu.make_async_copy(k_h.at[:, lsl(g)], k_v.at[:, lsl(g)], sems.at[3 * g]),
              pltpu.make_async_copy(v_h.at[:, lsl(g)], v_v.at[:, lsl(g)], sems.at[3 * g + 1]),
              pltpu.make_async_copy(ssmk_h.at[lsl(g), :], ssmk_v.at[lsl(g), :], sems.at[3 * g + 2])]
             for g in range(NG)]
    srcs = [wm_h, q_h, w1_h, w2_h, w3_h, w4_h]
    dsts = [wm_v, q_v, w1_v, w2_v, w3_v, w4_v]
    cps = [pltpu.make_async_copy(s, d, sems.at[3 * NG + i]) for i, (s, d) in enumerate(zip(srcs, dsts))]
    c_wm, c_q, c_w1, c_w2, c_w3, c_w4 = cps
    for cp in a_cps[0] + a_cps[1]:
        cp.start()

    sk = sk_ref[...].astype(F32)
    sd = sd_ref[...].astype(F32)
    fx = fk_ref[...]
    inv = inv_ref[...]
    nt = (((1,), (1,)), ((), ()))

    def fwd(g):
        ls = lsl(g)
        for cp in a_cps[g]:
            cp.wait()
        for cp in (a_cps[g + 2] if g + 2 < NG else []) + [[c_wm], [c_q, c_w1], [c_w2, c_w3], [c_w4], []][g]:
            cp.start()
        prev = None
        kf_s[g, 0:PAD, :] = jnp.zeros((PAD, 128), F32)
        kf_s[g, PAD:, :] = k_v[:, ls].astype(F32)
        for j in range(NC):
            r0 = j * C
            ks = kf_s[g, pl.ds(PAD + r0, C), :] * sk[0:1, ls]
            for s in range(1, 4):
                ks = ks + kf_s[g, pl.ds(PAD + r0 - s, C), :] * sk[s:s + 1, ls]
            kv = ks * v_v[pl.ds(r0, C), ls].astype(F32)
            xf_s[g, j] = _dot(fx, kv.astype(BF16))
            kq = jax.lax.dot_general(fx, ssmk_v[ls, pl.ds(r0, C)], nt, preferred_element_type=F32)
            sg = sgn_ref[...]
            if j == 0:
                kq_s[g, 0, 0:C, :] = -sg * kq[C:]
                kq_s[g, 0, C:, :] = sg * (kq[0:C] + sd[:, ls])
            else:
                kq_s[g, j, 0:C, :] = prev[0:C] - sg * kq[C:]
                kq_s[g, j, C:, :] = prev[C:] + sg * kq[0:C]
            prev = kq

    def conv(g, i0, re, im):
        acc = {}
        for j in range(i0 + 2):
            xr, xi = xf_s[g, j, re, :], xf_s[g, j, im, :]
            for i in range(max(i0, j), i0 + 2):
                kr, ki = kq_s[g, i - j, re, :], kq_s[g, i - j, im, :]
                if i in acc:
                    acc[i] = ((acc[i][0] + xr * kr) - xi * ki, (acc[i][1] + xr * ki) + xi * kr)
                else:
                    acc[i] = (xr * kr - xi * ki, xr * ki + xi * kr)
        for i in acc:
            yf_s[g, i, re, :] = acc[i][0].astype(BF16)
            yf_s[g, i, im, :] = acc[i][1].astype(BF16)

    def invf(g, i):
        y_s[i * C:(i + 1) * C, lsl(g)] = _dot(inv, yf_s[g, i]).astype(BF16)

    for g in range(NG):
        fwd(g)

        def freq_tile(p, carry, g=g):
            re = pl.ds(pl.multiple_of(p * 16, 16), 16)
            im = pl.ds(pl.multiple_of(C + p * 16, 16), 16)
            for i0 in range(0, NC, 2):
                conv(g, i0, re, im)
            return carry

        jax.lax.fori_loop(0, C // 16, freq_tile, 0)
        for i in range(NC):
            invf(g, i)

    c_wm.wait()
    cs = jax.nn.silu(c_ref[...].astype(F32)).astype(BF16)
    mod = _dot(jnp.broadcast_to(cs, (16, D)), wm_v[...])[0:1]
    sa, ca, ga, sb, cb, gb = [mod[:, i * D:(i + 1) * D] for i in range(6)]

    for cp in (c_q, c_w1, c_w2, c_w3, c_w4):
        cp.wait()

    for g in range(NG):
        h_s[g, 0:PAD, :] = jnp.zeros((PAD, 128), F32)
        h_s[g, PAD + S:, :] = jnp.zeros((PAD, 128), F32)

    def x1_hb(rows):
        q = q_v[rows, :].astype(F32)
        h = _ln(q) * (1.0 + ca) + sa
        x1 = q + ga * (h * y_s[rows, :].astype(F32))
        return x1, _ln(x1) * (1.0 + cb) + sb

    def b1(t, carry):
        r0 = t * TM if isinstance(t, int) else pl.multiple_of(t * TM, TM)
        _, hb = x1_hb(pl.ds(r0, TM))
        h = _gelu(_dot(_ln(hb).astype(BF16), w1_v[...]))
        for g in range(NG):
            h_s[g, pl.ds(PAD + r0, TM), :] = h[:, g * 128:(g + 1) * 128]
        return carry

    b1(0, 0)
    b1(1, 0)

    def out_cp(t):
        r0 = t * TM
        return pltpu.make_async_copy(o_v.at[pl.ds(r0, TM)], o_h.at[pl.ds(r0, TM)], osems.at[t])

    lane = jax.lax.broadcasted_iota(jnp.int32, (TM, 128), 1)

    def b2(t):
        r0 = t * TM
        x1, hb = x1_hb(pl.ds(r0, TM))
        ld = lambda g, off: h_s[g, pl.ds(PAD + r0 + off, TM), :]
        hs = jnp.concatenate([
            ld(0, -1),
            jnp.where(lane < 32, ld(1, -1), ld(1, 1)),
            jnp.where(lane < 64, ld(2, 1), ld(2, -2)),
            jnp.where(lane < 96, ld(3, -2), ld(3, 2)),
            ld(4, 2)], axis=1)
        if t + 2 < NT:
            b1(t + 2, 0)
        xb = hb + _dot(hs.astype(BF16), w2_v[...])
        lx = _ln(xb).astype(BF16)
        h2 = None
        for f0 in range(0, F, 896):
            f1 = min(F, f0 + 896)
            u = _gelu(jax.lax.dot_general(lx, w3_v[f0:f1, :], nt, preferred_element_type=F32))
            d = _dot(u.astype(BF16), w4_v[f0:f1, :])
            h2 = d if h2 is None else h2 + d
        o_v[pl.ds(r0, TM), :] = (x1 + gb * (xb + h2)).astype(BF16)
        out_cp(t).start()

    for t in range(NT):
        b2(t)
    for t in range(NT):
        out_cp(t).wait()


@jax.jit
def pallas_adaLN_cond__ssm_conv_h3__mixer_s_mlp__prompt_kernel(
    A_q, A_k, A_v, A_shift_k, A_ssm_k, A_ssm_D, B_x, B_w1, B_w2, B_w3, B_w4, c, w_mod,
):
    fk, inv, sgn = _dft_consts()
    hbm = pl.BlockSpec(memory_space=pl.ANY)
    vm = pl.BlockSpec(memory_space=pltpu.VMEM)
    V = pltpu.VMEM
    out = pl.pallas_call(
        _kernel,
        in_specs=[hbm, hbm, hbm, vm, hbm, vm, hbm, hbm, hbm, hbm, vm, hbm, vm, vm, vm],
        out_specs=hbm,
        out_shape=jax.ShapeDtypeStruct((S, D), BF16),
        scratch_shapes=[
            V((S, D), BF16), V((S, D), BF16), V((S, D), BF16), V((D, S), BF16),
            V((D, D), BF16), V((D, D), BF16), V((F, D), BF16), V((F, D), BF16),
            V((D, 6 * D), BF16), V((S, D), BF16),
            V((NG, PAD + S, 128), F32), *[V((NG, NC, 2 * C, 128), F32)] * 2,
            V((NG, NC, 2 * C, 128), BF16), V((S, D), BF16), V((NG, S + 2 * PAD, 128), F32),
            pltpu.SemaphoreType.DMA((3 * NG + 6,)), pltpu.SemaphoreType.DMA((NT,)),
        ],
        compiler_params=pltpu.CompilerParams(vmem_limit_bytes=100 * 1024 * 1024),
    )(A_q.reshape(S, D), A_k.reshape(S, D), A_v.reshape(S, D), A_shift_k.T, A_ssm_k,
      A_ssm_D.reshape(1, D), B_w1, B_w2, B_w3.T, B_w4, c, w_mod,
      jnp.asarray(fk[:, :C], BF16), jnp.asarray(inv, BF16), jnp.asarray(sgn, F32))
    return out.reshape(1, S, D)
```
